```python
import os as _os
_os.environ.setdefault("JAX_PLATFORMS", "cpu")
import jax
import jax.numpy as jnp

def _softmax(x, axis=-1):
    return jax.nn.softmax(x, axis=axis)
def _gelu(x):
    return jax.nn.gelu(x, approximate=True)
def _silu(x):
    return jax.nn.silu(x)
def _sigmoid(x):
    return jax.nn.sigmoid(x)
def _layernorm(x, axis=-1, eps=1e-5):
    m = jnp.mean(x, axis=axis, keepdims=True)
    v = jnp.var(x, axis=axis, keepdims=True)
    return (x - m) / jnp.sqrt(v + eps)
def _scatter_add(tgt, idx, src, axis=0):
    return tgt.at[idx].add(src)
def _segment_sum(src, seg, n):
    return jax.ops.segment_sum(src, seg, n)
class _Rng:
    def __init__(self, key):
        self._k = key
    def _next(self):
        self._k, sub = jax.random.split(self._k)
        return sub
    def normal(self, shape):
        return jax.random.normal(self._next(), shape, dtype=jnp.bfloat16)
    def randint(self, lo, hi, shape):
        return jax.random.randint(self._next(), shape, lo, hi, dtype=jnp.int32)
    def uniform(self, shape, lo=0.0, hi=1.0):
        return jax.random.uniform(self._next(), shape, jnp.bfloat16, lo, hi)
    def permutation(self, n):
        return jax.random.permutation(self._next(), n)


kernel_name = 'gated_mix__compressed_kv_cla__linear_attn_block__prompt'

def setup_inputs():
    _rng = _Rng(jax.random.key(int.from_bytes(__import__("os").urandom(4), "little")))
    _w = (lambda a: (lambda t: t.astype(jnp.bfloat16) if jnp.issubdtype(t.dtype, jnp.floating) else t)(jnp.asarray(a)))
    def _A_setup():
        B, H, Sq, Sk, D, M = 1, 16, 2048, 2048, 256, 448
        Dc = 4 * D
        return {
            "x": _w((lambda *s: _rng.normal(s) * 0.05)(B, Sq, M)),
            "c_kv": _w((lambda *s: _rng.normal(s) * 0.8)(B, Sk, Dc)),
            "w_q": _w((lambda *s: _rng.normal(s) * 3.2)(M, H, D) * (M ** -0.5)),
            "w_uk": _w((lambda *s: _rng.normal(s) * 3.2)(Dc, H, D) * (Dc ** -0.5)),
            "w_uv": _w((lambda *s: _rng.normal(s) * 0.8)(Dc, H, D) * (Dc ** -0.5)),
            "w_o": _w((lambda *s: _rng.normal(s) * 0.8)(H, D, M) * ((H * D) ** -0.5)),
        }
    _A_in = _A_setup()

    def _B_setup():
        B, S, D = 1, 2048, 448
        return {
            "x": _w((lambda *s: _rng.normal(s) * 0.05)(B, S, D)),
            "wqkv": _w((lambda *s: _rng.normal(s) * 1.6)(D, 3 * D)),
            "wo": _w((lambda *s: _rng.normal(s) * 0.4)(D, D)),
        }
    _B_in = _B_setup()

    return {
        "A_x": _A_in["x"],
        "A_c_kv": _A_in["c_kv"],
        "A_w_q": _A_in["w_q"],
        "A_w_uk": _A_in["w_uk"],
        "A_w_uv": _A_in["w_uv"],
        "A_w_o": _A_in["w_o"],
        "B_x": _B_in["x"],
        "B_wqkv": _B_in["wqkv"],
        "B_wo": _B_in["wo"],
        "gate_w": _w((lambda *s: _rng.normal(s) * 0.05)(448) * 16.0),
    }

def reference(A_x, A_c_kv, A_w_q, A_w_uk, A_w_uv, A_w_o, B_x, B_wqkv, B_wo, gate_w):
    def _A_ref(x, c_kv, w_q, w_uk, w_uv, w_o):
        B, Sq, M = x.shape[0], x.shape[1], x.shape[2]
        Sk = c_kv.shape[1]
        H, D = w_q.shape[1], w_q.shape[2]
        q = jnp.einsum("bqm,mhd->bhqd", x, w_q)
        k = jnp.einsum("bkc,chd->bhkd", c_kv, w_uk)
        v = jnp.einsum("bkc,chd->bhkd", c_kv, w_uv)
        scores = jnp.einsum("bhqd,bhkd->bhqk", q, k) * (D ** -0.5)
        off = Sk - Sq
        qi = jnp.arange(Sq)[:, None]
        kj = jnp.arange(Sk)[None, :]
        cmask = kj <= (qi + off)
        scores = jnp.where(cmask[None, None], scores, -1e9)
        p = _softmax(scores, axis=-1)
        ctx = jnp.einsum("bhqk,bhkd->bhqd", p, v)
        return jnp.einsum("bhqd,hdm->bqm", ctx, w_o)

    def _B_ref(x, wqkv, wo):
        B, S, D = x.shape
        H = 16; Dh = D // H
        qkv = (lambda x, *d: x.transpose(*d))((x @ wqkv).reshape(B, S, 3, H, Dh), 2, 0, 3, 1, 4)
        q, k, v = qkv[0], qkv[1], qkv[2]
        phi = lambda t: jnp.where(t > 0, t + 1, jnp.exp(t)) + 1e-6
        pq, pk = phi(q), phi(k)
        kv = jnp.einsum("bhsd,bhse->bhde", pk, v)
        z = jnp.einsum("bhsd->bhd", pk)
        num = jnp.einsum("bhqd,bhde->bhqe", pq, kv)
        den = jnp.einsum("bhqd,bhd->bhq", pq, z)[..., None] + 1e-6
        o = num / den
        return (lambda x, *d: x.transpose(*d))(o, 0, 2, 1, 3).reshape(B, S, D) @ wo

    x = A_x
    g = _sigmoid((x * gate_w).sum(-1, keepdims=True))
    a = _A_ref(x, A_c_kv, A_w_q, A_w_uk, A_w_uv, A_w_o)
    b = _B_ref(x, B_wqkv, B_wo)
    return g * a + (1 - g) * b
```

```python
import functools

import jax
import jax.numpy as jnp
import jax.experimental.pallas as pl
import jax.experimental.pallas.tpu as pltpu

_NT = (((1,), (1,)), ((), ()))
_NN = (((1,), (0,)), ((), ()))
_TN = (((0,), (0,)), ((), ()))


def _dot(a, b, dims=_NN):
    return jax.lax.dot_general(a, b, dims, preferred_element_type=jnp.float32)


def _kernel(xt_ref, c_hbm, wq_hbm, wuk_hbm, wuv_hbm, wot_ref, wqkv_ref, bwo_ref,
            gw_ref, o_ref,
            c_s, wq_b, wuk_b, wuv_b, wsem, csem,
            x_s, wq_s, wuk_s, wuv_s, q_s, k_s, v_s, acc_s,
            bg_s, g_s, wt_s, bwot_s, pq_s, kv_s, z_s, kvz_s,
            *, S, M, D, Dc, H, HB, tq, tp, tb, tk):
    h = pl.program_id(0)
    bf16 = jnp.bfloat16
    f32 = jnp.float32
    u32 = jnp.uint32
    scale = D ** -0.5

    def w_copies(hh, slot):
        hp = hh // 2
        base = (hp // 4) * 8 + hp % 4
        cps = []
        for mi, (src, dst) in enumerate(((wq_hbm, wq_b), (wuk_hbm, wuk_b), (wuv_hbm, wuv_b))):
            s32 = src.bitcast(u32)
            for dt in range(2):
                cps.append(pltpu.make_async_copy(
                    s32.at[:, base + dt * 4, :],
                    dst.at[slot, :, pl.ds(dt * 128, 128)],
                    wsem.at[slot, mi, dt]))
        return cps

    c_copy = pltpu.make_async_copy(c_hbm, c_s, csem)

    @pl.when(h == 0)
    def _():
        for cp in w_copies(0, 0):
            cp.start()
        c_copy.start()

        Dh = M // HB

        def phi(t):
            return jnp.where(t > 0, t + 1.0, jnp.exp(t)) + 1e-6

        wt_s[...] = wqkv_ref[...].T
        bwot_s[...] = bwo_ref[...].T
        kv_s[...] = jnp.zeros(kv_s.shape, f32)
        z_s[...] = jnp.zeros(z_s.shape, f32)
        acc_s[...] = jnp.zeros(acc_s.shape, f32)
        gw8 = jnp.broadcast_to(gw_ref[...], (8, M))
        ones8 = jnp.ones((8, tb), bf16)

        def p1(j, carry):
            cols = pl.ds(pl.multiple_of(j * tb, tb), tb)
            xt = xt_ref[:, cols]
            x_s[cols, :] = xt.T
            g_s[:, cols] = jax.nn.sigmoid(_dot(gw8, xt))
            qb = _dot(wt_s[0:M, :], xt).astype(bf16).astype(f32)
            kb = _dot(wt_s[M:2 * M, :], xt).astype(bf16).astype(f32)
            vb = _dot(wt_s[2 * M:3 * M, :], xt).astype(bf16)
            pq_s[:, cols] = phi(qb).astype(bf16)
            pk = phi(kb).astype(bf16)
            kv_s[...] += _dot(vb, pk, _NT)
            z_s[...] += _dot(ones8, pk, _NT)
            return carry

        jax.lax.fori_loop(0, S // tb, p1, 0)

        rh = jax.lax.broadcasted_iota(jnp.int32, (M, M), 0) // Dh
        ch = jax.lax.broadcasted_iota(jnp.int32, (M, M), 1) // Dh
        same = rh == ch
        kvz_s[0:M, :] = jnp.where(same, kv_s[...], 0.0).astype(bf16)
        kvz_s[M:2 * M, :] = jnp.where(same, z_s[0:1, :], 0.0).astype(bf16)

        def p2(j, carry):
            cols = pl.ds(pl.multiple_of(j * tb, tb), tb)
            pq = pq_s[:, cols]
            num = _dot(kvz_s[0:M, :], pq)
            den = _dot(kvz_s[M:2 * M, :], pq) + 1e-6
            o = (num / den).astype(bf16)
            b = _dot(bwot_s[...], o)
            bg_s[:, cols] = (1.0 - g_s[0:1, cols]) * b
            return carry

        jax.lax.fori_loop(0, S // tb, p2, 0)
        c_copy.wait()

    slot = h % 2
    for cp in w_copies(h, slot):
        cp.wait()

    @pl.when(h + 1 < H)
    def _():
        for cp in w_copies(h + 1, 1 - slot):
            cp.start()

    sh = (1 - (h % 2)).astype(u32) * 16

    def unpack(b_ref):
        u = (b_ref[slot] << sh) & u32(0xFFFF0000)
        return pltpu.bitcast(u, f32).astype(bf16)

    wq_s[...] = unpack(wq_b)
    wuk_s[...] = unpack(wuk_b)
    wuv_s[...] = unpack(wuv_b)

    row_i = jax.lax.broadcasted_iota(jnp.int32, (tq, tq // 2), 0)
    col_i = jax.lax.broadcasted_iota(jnp.int32, (tq, tq // 2), 1)
    tri = col_i <= row_i

    for r in range(S // tp):
        prow = pl.ds(r * tp, tp)
        q_s[prow, :] = (_dot(x_s[prow, :], wq_s[...]) * scale).astype(bf16)
        c = c_s[prow, :]
        k_s[prow, :] = _dot(c, wuk_s[...]).astype(bf16)
        v_s[prow, :] = _dot(c, wuv_s[...]).astype(bf16)

    def chunks_of(i):
        chunks = []
        st = 0
        while st < i * tq:
            sz = min(tk, i * tq - st)
            chunks.append((st, sz))
            st += sz
        return chunks

    hq = tq // 2

    def stage1(i):
        r0 = i * tq
        q = q_s[pl.ds(r0, tq), :]
        ss = []
        m = None
        for (st, sz) in chunks_of(i):
            s_c = _dot(q, k_s[pl.ds(st, sz), :], _NT)
            mc = jnp.max(s_c, axis=-1, keepdims=True)
            m = mc if m is None else jnp.maximum(m, mc)
            ss.append(s_c)
        s0 = _dot(q, k_s[pl.ds(r0, hq), :], _NT)
        s0 = jnp.where(tri, s0, -1e9)
        mc = jnp.max(s0, axis=-1, keepdims=True)
        m = mc if m is None else jnp.maximum(m, mc)
        ss.append(s0)
        s1 = _dot(q_s[pl.ds(r0 + hq, hq), :], k_s[pl.ds(r0 + hq, hq), :], _NT)
        s1 = jnp.where(tri[:hq], s1, -1e9)
        m1 = jnp.maximum(m[hq:], jnp.max(s1, axis=-1, keepdims=True))
        m = jnp.concatenate([m[:hq], m1], axis=0)
        return ss, s1, m

    def stage2(i, ss, s1, m):
        r0 = i * tq
        l = None
        ctx = None
        for s_c, (st, sz) in zip(ss, chunks_of(i) + [(r0, hq)]):
            p = jnp.exp(s_c - m)
            lc = jnp.sum(p, axis=-1, keepdims=True)
            l = lc if l is None else l + lc
            cc = _dot(p.astype(bf16), v_s[pl.ds(st, sz), :])
            ctx = cc if ctx is None else ctx + cc
        p1 = jnp.exp(s1 - m[hq:])
        l1 = l[hq:] + jnp.sum(p1, axis=-1, keepdims=True)
        c1 = ctx[hq:] + _dot(p1.astype(bf16), v_s[pl.ds(r0 + hq, hq), :])
        l = jnp.concatenate([l[:hq], l1], axis=0)
        ctx = jnp.concatenate([ctx[:hq], c1], axis=0)
        return ctx, l

    def stage3(i, ctx, l):
        rows = pl.ds(i * tq, tq)
        ctx = (ctx / l).astype(bf16)
        acc_s[:, rows] += _dot(wot_ref[...], ctx, _NT)

    order = list(reversed(range(S // tq)))
    n = len(order)
    r1, r2 = {}, {}
    for t in range(n + 2):
        if t < n:
            r1[t] = stage1(order[t])
        if 0 <= t - 2 < n:
            stage3(order[t - 2], *r2.pop(t - 2))
        if 0 <= t - 1 < n:
            r2[t - 1] = stage2(order[t - 1], *r1.pop(t - 1))

    @pl.when(h == H - 1)
    def _():
        o_ref[...] = (g_s[0:1, :] * acc_s[...] + bg_s[...]).astype(o_ref.dtype)


def _tile_view(w):
    C = w.shape[0]
    return w.reshape(C, 2, 8, 2, 128).transpose(0, 1, 3, 2, 4).reshape(C, 32, 128)


@jax.jit
def pallas_gated_mix__compressed_kv_cla__linear_attn_block__prompt_kernel(
    A_x: jax.Array,
    A_c_kv: jax.Array,
    A_w_q: jax.Array,
    A_w_uk: jax.Array,
    A_w_uv: jax.Array,
    A_w_o: jax.Array,
    B_x: jax.Array,
    B_wqkv: jax.Array,
    B_wo: jax.Array,
    gate_w: jax.Array,
):
    B, S, M = A_x.shape
    Dc = A_c_kv.shape[-1]
    _, H, D = A_w_q.shape
    HB = 16
    xt = A_x.reshape(S, M).T
    c = A_c_kv.reshape(S, Dc)
    wq = _tile_view(A_w_q)
    wuk = _tile_view(A_w_uk)
    wuv = _tile_view(A_w_uv)
    wot = jnp.swapaxes(A_w_o, 1, 2)
    gw = gate_w.reshape(1, M)

    bf16, f32, u32 = jnp.bfloat16, jnp.float32, jnp.uint32
    kern = functools.partial(_kernel, S=S, M=M, D=D, Dc=Dc, H=H, HB=HB,
                             tq=256, tp=512, tb=512, tk=512)
    out_t = pl.pallas_call(
        kern,
        grid=(H,),
        in_specs=[
            pl.BlockSpec((M, S), lambda h: (0, 0)),
            pl.BlockSpec(memory_space=pl.ANY),
            pl.BlockSpec(memory_space=pl.ANY),
            pl.BlockSpec(memory_space=pl.ANY),
            pl.BlockSpec(memory_space=pl.ANY),
            pl.BlockSpec((None, M, D), lambda h: (h, 0, 0)),
            pl.BlockSpec((M, 3 * M), lambda h: (0, 0)),
            pl.BlockSpec((M, M), lambda h: (0, 0)),
            pl.BlockSpec((1, M), lambda h: (0, 0)),
        ],
        out_specs=pl.BlockSpec((M, S), lambda h: (0, 0)),
        out_shape=jax.ShapeDtypeStruct((M, S), A_x.dtype),
        scratch_shapes=[
            pltpu.VMEM((S, Dc), bf16),
            pltpu.VMEM((2, M, D), u32),
            pltpu.VMEM((2, Dc, D), u32),
            pltpu.VMEM((2, Dc, D), u32),
            pltpu.SemaphoreType.DMA((2, 3, 2)),
            pltpu.SemaphoreType.DMA(()),
            pltpu.VMEM((S, M), bf16),
            pltpu.VMEM((M, D), bf16),
            pltpu.VMEM((Dc, D), bf16),
            pltpu.VMEM((Dc, D), bf16),
            pltpu.VMEM((S, D), bf16),
            pltpu.VMEM((S, D), bf16),
            pltpu.VMEM((S, D), bf16),
            pltpu.VMEM((M, S), f32),
            pltpu.VMEM((M, S), f32),
            pltpu.VMEM((8, S), f32),
            pltpu.VMEM((3 * M, M), bf16),
            pltpu.VMEM((M, M), bf16),
            pltpu.VMEM((M, S), bf16),
            pltpu.VMEM((M, M), f32),
            pltpu.VMEM((8, M), f32),
            pltpu.VMEM((2 * M, M), bf16),
        ],
        compiler_params=pltpu.CompilerParams(
            dimension_semantics=("arbitrary",),
            vmem_limit_bytes=100 * 1024 * 1024,
        ),
    )(xt, c, wq, wuk, wuv, wot, B_wqkv, B_wo, gw)
    return out_t.T.reshape(B, S, M)
```

```python
import functools

import jax
import jax.numpy as jnp
import jax.experimental.pallas as pl
import jax.experimental.pallas.tpu as pltpu

_NT = (((1,), (1,)), ((), ()))
_NN = (((1,), (0,)), ((), ()))
_TN = (((0,), (0,)), ((), ()))

_SCHED = (
    (0, 0), (0, 1), (1, 1), (1, 0), (0, 2), (2, 1), (2, 0), (1, 3), (1, 2),
    (0, 3), (3, 1), (3, 0), (2, 3), (2, 2), (1, 7), (1, 6), (2, 7), (1, 5),
    (2, 6), (1, 4), (3, 7), (2, 5), (3, 6), (2, 4), (3, 3), (3, 2), (3, 5),
    (3, 4),
)


def _dot(a, b, dims=_NN):
    return jax.lax.dot_general(a, b, dims, preferred_element_type=jnp.float32)


def _kernel(xt_hbm, c_hbm, wq_hbm, wuk_hbm, wuv_hbm, wot_hbm, wqkv_ref, bwo_hbm,
            gw_ref, o_hbm,
            c_s, wq_b, wuk_b, wuv_b, xt_s, bwo_s, wot_s, ob_s,
            wsem, xsem, osem, msem,
            x_s, wq_s, wuk_s, wuv_s, q_s, k_s, v_s, acc_s,
            g_s, wt_s, w2_s, pq_s, kv_s, z_s, kvz_s,
            *, S, M, D, H, HB, tq, tp, tb, tb2, tk):
    h = pl.program_id(0)
    bf16 = jnp.bfloat16
    f32 = jnp.float32
    u32 = jnp.uint32
    scale = D ** -0.5
    Dh = M // HB

    def w_copies(hh, slot):
        hp = hh // 2
        base = (hp // 4) * 8 + hp % 4
        cps = []
        for mi, (src, dst) in enumerate(
                ((wq_hbm, wq_b), (wuk_hbm, wuk_b), (wuv_hbm, wuv_b))):
            s32 = src.bitcast(u32)
            for dt in range(2):
                cps.append(pltpu.make_async_copy(
                    s32.at[:, base + dt * 4, :],
                    dst.at[slot, :, pl.ds(dt * 128, 128)],
                    wsem.at[slot * 6 + mi * 2 + dt]))
        return cps

    tiles = []
    for d0 in range(0, M, 128):
        d1 = min(d0 + 128, M)
        e0 = (d0 // Dh) * Dh
        e1 = ((d1 - 1) // Dh + 1) * Dh
        tiles.append((d0, d1, (e0 // 16) * 16, min(-(-e1 // 16) * 16, M)))

    @pl.when(h == 0)
    def _():
        def x_copy(j):
            cols = pl.ds(pl.multiple_of(j * tb, tb), tb)
            return pltpu.make_async_copy(
                xt_hbm.at[:, cols], xt_s.at[:, cols], xsem.at[j])

        b_copy = pltpu.make_async_copy(bwo_hbm, bwo_s, msem.at[0])
        c_copy = pltpu.make_async_copy(c_hbm, c_s, msem.at[1])
        t_copy = pltpu.make_async_copy(wot_hbm, wot_s, msem.at[2])
        for j in range(S // tb):
            x_copy(j).start()
        b_copy.start()
        for cp in w_copies(0, 0):
            cp.start()
        c_copy.start()
        t_copy.start()

        def phi(t):
            return jnp.where(t > 0, t + 1.0, jnp.exp(t)) + 1e-6

        wt_s[...] = wqkv_ref[...].T
        kv_s[...] = jnp.zeros(kv_s.shape, f32)
        z_s[...] = jnp.zeros(z_s.shape, f32)
        gw8 = jnp.broadcast_to(gw_ref[...].reshape(1, M), (8, M))
        ones8 = jnp.ones((8, tb), bf16)

        def p1(j, carry):
            cols = pl.ds(pl.multiple_of(j * tb, tb), tb)
            x_copy(j).wait()
            xt = xt_s[:, cols]
            x_s[cols, :] = xt.T
            g_s[:, cols] = jax.nn.sigmoid(_dot(gw8, xt))
            qb = _dot(wt_s[0:M, :], xt).astype(bf16).astype(f32)
            kb = _dot(wt_s[M:2 * M, :], xt).astype(bf16).astype(f32)
            vb = _dot(wt_s[2 * M:3 * M, :], xt).astype(bf16)
            pq_s[:, cols] = phi(qb).astype(bf16)
            pk = phi(kb).astype(bf16)
            for (d0, d1, e0, e1) in tiles:
                kv_s[e0:e1, d0:d1] += _dot(vb[e0:e1], pk[d0:d1], _NT)
            z_s[...] += _dot(ones8, pk, _NT)
            return carry

        jax.lax.fori_loop(0, S // tb, p1, 0)
        b_copy.wait()
        c_copy.wait()
        t_copy.wait()

    slot = h % 2
    for cp in w_copies(h, slot):
        cp.wait()

    @pl.when(h + 1 < H)
    def _():
        for cp in w_copies(h + 1, 1 - slot):
            cp.start()

    sh = (1 - (h % 2)).astype(u32) * 16

    def unpack(b_ref):
        u = (b_ref[slot] << sh) & u32(0xFFFF0000)
        return pltpu.bitcast(u, f32).astype(bf16)

    wq_s[...] = unpack(wq_b)
    wuk_s[...] = unpack(wuk_b)
    wuv_s[...] = unpack(wuv_b)

    hq = tq // 2
    row_i = jax.lax.broadcasted_iota(jnp.int32, (tq, hq), 0)
    col_i = jax.lax.broadcasted_iota(jnp.int32, (tq, hq), 1)
    tri = col_i <= row_i

    def stage0(r):
        prow = pl.ds(r * tp, tp)
        q_s[prow, :] = (_dot(x_s[prow, :], wq_s[...]) * scale).astype(bf16)
        c = c_s[prow, :]
        k_s[prow, :] = _dot(c, wuk_s[...]).astype(bf16)
        v_s[prow, :] = _dot(c, wuv_s[...]).astype(bf16)

    def chunks_of(i):
        return [(st, min(tk, i * tq - st)) for st in range(0, i * tq, tk)]

    def stage1(i):
        r0 = i * tq
        q = q_s[pl.ds(r0, tq), :]
        ss = []
        m = None
        for (st, sz) in chunks_of(i):
            s_c = _dot(q, k_s[pl.ds(st, sz), :], _NT)
            mc = jnp.max(s_c, axis=-1, keepdims=True)
            m = mc if m is None else jnp.maximum(m, mc)
            ss.append(s_c)
        s0 = _dot(q, k_s[pl.ds(r0, hq), :], _NT)
        s0 = jnp.where(tri, s0, -1e9)
        mc = jnp.max(s0, axis=-1, keepdims=True)
        m = mc if m is None else jnp.maximum(m, mc)
        ss.append(s0)
        s1 = _dot(q_s[pl.ds(r0 + hq, hq), :], k_s[pl.ds(r0 + hq, hq), :], _NT)
        s1 = jnp.where(tri[:hq], s1, -1e9)
        m1 = jnp.maximum(m[hq:], jnp.max(s1, axis=-1, keepdims=True))
        m = jnp.concatenate([m[:hq], m1], axis=0)
        return ss, s1, m

    def stage2(i, ss, s1, m):
        r0 = i * tq
        l = None
        ctx = None
        for s_c, (st, sz) in zip(ss, chunks_of(i) + [(r0, hq)]):
            p = jnp.exp(s_c - m).astype(bf16)
            lc = jnp.sum(p.astype(f32), axis=-1, keepdims=True)
            l = lc if l is None else l + lc
            cc = _dot(p, v_s[pl.ds(st, sz), :])
            ctx = cc if ctx is None else ctx + cc
        p1 = jnp.exp(s1 - m[hq:]).astype(bf16)
        l1 = l[hq:] + jnp.sum(p1.astype(f32), axis=-1, keepdims=True)
        c1 = ctx[hq:] + _dot(p1, v_s[pl.ds(r0 + hq, hq), :])
        l = jnp.concatenate([l[:hq], l1], axis=0)
        ctx = jnp.concatenate([ctx[:hq], c1], axis=0)
        return ctx, l

    def stage3(i, ctx, l):
        rows = pl.ds(i * tq, tq)
        ctx = (ctx / l).astype(bf16)
        prev = jnp.where(h > 0, acc_s[:, rows], 0.0)
        acc_s[:, rows] = prev + _dot(wot_s[h], ctx, _NT)

    r1, r2 = {}, {}
    for st, i in _SCHED:
        if st == 0:
            stage0(i)
        elif st == 1:
            r1[i] = stage1(i)
        elif st == 2:
            r2[i] = stage2(i, *r1.pop(i))
        else:
            stage3(i, *r2.pop(i))

    @pl.when(h == H - 1)
    def _():
        def o_copy(j):
            cols = pl.ds(j * tb2, tb2)
            return pltpu.make_async_copy(
                ob_s.at[:, cols], o_hbm.at[:, cols], osem.at[j])

        rh = jax.lax.broadcasted_iota(jnp.int32, (M, M), 0) // Dh
        ch = jax.lax.broadcasted_iota(jnp.int32, (M, M), 1) // Dh
        kvz_s[...] = jnp.where(rh == ch, kv_s[...], 0.0).astype(bf16)
        hr = jax.lax.broadcasted_iota(jnp.int32, (HB, M), 0)
        hc = jax.lax.broadcasted_iota(jnp.int32, (HB, M), 1) // Dh
        zh = jnp.where(hr == hc, z_s[0:1, :], 0.0).astype(bf16)
        er = jax.lax.broadcasted_iota(jnp.int32, (M, 2 * HB), 0) // Dh
        ec = jax.lax.broadcasted_iota(jnp.int32, (M, 2 * HB), 1) % HB
        e2 = jnp.where(er == ec, 1.0, 0.0).astype(bf16)

        for (d0, d1, e0, e1) in tiles:
            w2_s[:, d0:d1] = _dot(
                bwo_s[e0:e1, :], kvz_s[e0:e1, d0:d1], _TN).astype(bf16)

        rden = 1.0 / (_dot(zh, pq_s[...]) + 1e-6)
        r_hi = rden.astype(bf16)
        r_lo = (rden - r_hi.astype(f32)).astype(bf16)
        rr = jnp.concatenate([r_hi, r_lo], axis=0)
        nj = S // tb2
        pqn = {}
        for j in range(nj + 1):
            if j < nj:
                cols = pl.ds(j * tb2, tb2)
                rexp = _dot(e2, rr[:, j * tb2:(j + 1) * tb2])
                pqn[j] = (pq_s[:, cols].astype(f32) * rexp).astype(bf16)
            if j > 0:
                cols = pl.ds((j - 1) * tb2, tb2)
                b = _dot(w2_s[...], pqn.pop(j - 1))
                g = g_s[0:1, cols]
                ob_s[:, cols] = (
                    g * acc_s[:, cols] + (1.0 - g) * b).astype(ob_s.dtype)
                o_copy(j - 1).start()
        for j in range(nj):
            o_copy(j).wait()


def _tile_view(w):
    C = w.shape[0]
    return w.reshape(C, 2, 8, 2, 128).transpose(0, 1, 3, 2, 4).reshape(C, 32, 128)


@jax.jit
def pallas_gated_mix__compressed_kv_cla__linear_attn_block__prompt_kernel(
    A_x: jax.Array,
    A_c_kv: jax.Array,
    A_w_q: jax.Array,
    A_w_uk: jax.Array,
    A_w_uv: jax.Array,
    A_w_o: jax.Array,
    B_x: jax.Array,
    B_wqkv: jax.Array,
    B_wo: jax.Array,
    gate_w: jax.Array,
):
    B, S, M = A_x.shape
    Dc = A_c_kv.shape[-1]
    _, H, D = A_w_q.shape
    HB = 16
    tq, tp, tb, tb2, tk = 256, 512, 512, 512, 256
    assert (B, S, H, D) == (1, 2048, 16, 256) and M % HB == 0

    xt = A_x.reshape(S, M).T
    c = A_c_kv.reshape(S, Dc)
    wq = _tile_view(A_w_q)
    wuk = _tile_view(A_w_uk)
    wuv = _tile_view(A_w_uv)
    wot = jnp.swapaxes(A_w_o, 1, 2)

    bf16, f32, u32 = jnp.bfloat16, jnp.float32, jnp.uint32
    kern = functools.partial(_kernel, S=S, M=M, D=D, H=H, HB=HB,
                             tq=tq, tp=tp, tb=tb, tb2=tb2, tk=tk)
    hbm = pl.BlockSpec(memory_space=pl.ANY)
    out_t = pl.pallas_call(
        kern,
        grid=(H,),
        in_specs=[
            hbm, hbm, hbm, hbm, hbm, hbm,
            pl.BlockSpec((M, 3 * M), lambda h: (0, 0)),
            hbm,
            pl.BlockSpec((M,), lambda h: (0,)),
        ],
        out_specs=hbm,
        out_shape=jax.ShapeDtypeStruct((M, S), A_x.dtype),
        scratch_shapes=[
            pltpu.VMEM((S, Dc), bf16),
            pltpu.VMEM((2, M, D), u32),
            pltpu.VMEM((2, Dc, D), u32),
            pltpu.VMEM((2, Dc, D), u32),
            pltpu.VMEM((M, S), bf16),
            pltpu.VMEM((M, M), bf16),
            pltpu.VMEM((H, M, D), bf16),
            pltpu.VMEM((M, S), A_x.dtype),
            pltpu.SemaphoreType.DMA((12,)),
            pltpu.SemaphoreType.DMA((S // tb,)),
            pltpu.SemaphoreType.DMA((S // tb2,)),
            pltpu.SemaphoreType.DMA((3,)),
            pltpu.VMEM((S, M), bf16),
            pltpu.VMEM((M, D), bf16),
            pltpu.VMEM((Dc, D), bf16),
            pltpu.VMEM((Dc, D), bf16),
            pltpu.VMEM((S, D), bf16),
            pltpu.VMEM((S, D), bf16),
            pltpu.VMEM((S, D), bf16),
            pltpu.VMEM((M, S), f32),
            pltpu.VMEM((8, S), f32),
            pltpu.VMEM((3 * M, M), bf16),
            pltpu.VMEM((M, M), bf16),
            pltpu.VMEM((M, S), bf16),
            pltpu.VMEM((M, M), f32),
            pltpu.VMEM((8, M), f32),
            pltpu.VMEM((M, M), bf16),
        ],
        compiler_params=pltpu.CompilerParams(
            dimension_semantics=("arbitrary",),
            vmem_limit_bytes=100 * 1024 * 1024,
        ),
    )(xt, c, wq, wuk, wuv, wot, B_wqkv, B_wo, gate_w)
    return out_t.T.reshape(B, S, M)
```
